```python
import os as _os
_os.environ.setdefault("JAX_PLATFORMS", "cpu")
import jax
import jax.numpy as jnp

def _softmax(x, axis=-1):
    return jax.nn.softmax(x, axis=axis)
def _gelu(x):
    return jax.nn.gelu(x, approximate=True)
def _silu(x):
    return jax.nn.silu(x)
def _sigmoid(x):
    return jax.nn.sigmoid(x)
def _layernorm(x, axis=-1, eps=1e-5):
    m = jnp.mean(x, axis=axis, keepdims=True)
    v = jnp.var(x, axis=axis, keepdims=True)
    return (x - m) / jnp.sqrt(v + eps)
def _scatter_add(tgt, idx, src, axis=0):
    return tgt.at[idx].add(src)
def _segment_sum(src, seg, n):
    return jax.ops.segment_sum(src, seg, n)
class _Rng:
    def __init__(self, key):
        self._k = key
    def _next(self):
        self._k, sub = jax.random.split(self._k)
        return sub
    def normal(self, shape):
        return jax.random.normal(self._next(), shape, dtype=jnp.bfloat16)
    def randint(self, lo, hi, shape):
        return jax.random.randint(self._next(), shape, lo, hi, dtype=jnp.int32)
    def uniform(self, shape, lo=0.0, hi=1.0):
        return jax.random.uniform(self._next(), shape, jnp.bfloat16, lo, hi)
    def permutation(self, n):
        return jax.random.permutation(self._next(), n)


kernel_name = 'standalone__cross_network_dcn_v2__recsys'

def setup_inputs():
    _rng = _Rng(jax.random.key(int.from_bytes(__import__("os").urandom(4), "little")))
    _w = (lambda a: (lambda t: t.astype(jnp.bfloat16) if jnp.issubdtype(t.dtype, jnp.floating) else t)(jnp.asarray(a)))
    B, F, D, L = 16384, 26, 16, 6
    Din = min(F * D, 512)
    R = max(Din // 4, 2)
    sc = Din ** -0.5
    return {
        "x0": _w((lambda *s: _rng.normal(s) * 0.05)(B, Din)),
        "U":  _w((lambda *s: _rng.normal(s) * 1.6)(L, Din, R) * sc),
        "V":  _w((lambda *s: _rng.normal(s) * 1.6)(L, R, Din) * sc),
        "bs": _w((lambda *s: _rng.normal(s) * 0.05)(L, Din)),
    }

def reference(x0, U, V, bs):
    x = x0
    for l in range(U.shape[0]):
        h = jnp.einsum('rd,bd->br', V[l], x)
        h = jnp.einsum('dr,br->bd', U[l], h)
        x = x0 * (h + bs[l]) + x
    return x
```

```python
import jax
import jax.numpy as jnp
from jax import lax
import jax.experimental.pallas as pl
import jax.experimental.pallas.tpu as pltpu

F32, BF16, U32 = jnp.float32, jnp.bfloat16, jnp.uint32


def _mm(a, b, dims=(((1,), (0,)), ((), ()))):
    return lax.dot_general(a, b, dims, preferred_element_type=F32)


@jax.jit
def pallas_standalone__cross_network_dcn_v2__recsys_kernel(
    x0: jax.Array,
    U: jax.Array,
    V: jax.Array,
    bs: jax.Array,
):
    B, D = x0.shape
    L, _, R = U.shape
    KM = 384
    NT = 4
    CN = NT * 128
    NV = 8
    NC = B // CN
    FIRST, BODY = 1, 3
    nf, nb = 2 * FIRST, 2 * BODY
    nsteps = 1 + (NC - nf) // nb
    W2 = 2
    OSPLIT = 4
    obounds = [(D * k // OSPLIT) // 16 * 16 for k in range(OSPLIT)] + [D]

    def kernel(x_hbm, u_hbm, v_hbm, b_hbm, o_hbm, xa0, xa1, xb0, xb1,
               xin, xout, ubuf, vbuf, vf_ref, uw_ref, vc_ref, bb_ref, bbuf, zero_ref, isem, osem, wsem):
        xs_refs = [[xa0, xa1], [xb0, xb1]]
        step = pl.program_id(0)

        def in_copy(c, sem):
            src = min(c, NC - 1) if isinstance(c, int) else jnp.minimum(c, NC - 1)
            return pltpu.make_async_copy(
                x_hbm.at[:, pl.ds(pl.multiple_of(src * CN, CN), CN)], xin.at[c], sem)

        def out_copy(c, k):
            r0, r1 = obounds[k], obounds[k + 1]
            return pltpu.make_async_copy(
                xout.at[c, r0:r1, :], o_hbm.at[r0:r1, pl.ds(pl.multiple_of(c * CN, CN), CN)], osem.at[0])

        def w_copies(l0, l1, k):
            return [pltpu.make_async_copy(v_hbm.at[l0:l1], vbuf.at[l0:l1], wsem.at[k]),
                    pltpu.make_async_copy(u_hbm.at[l0:l1], ubuf.at[l0:l1], wsem.at[k])]

        group0 = (w_copies(0, W2, 0) + [pltpu.make_async_copy(b_hbm, bbuf, wsem.at[0])]
                  + [in_copy(c, wsem.at[0]) for c in range(2)])
        group1 = w_copies(W2, L, 1)

        @pl.when(step == 0)
        def _():
            for cp in group0:
                cp.start()
            zero_ref[0] = 0
            zero_ref[1] = 0

        iw = zero_ref[0]
        ir = zero_ref[1]

        def prep(l):
            vf = vbuf[l].astype(F32)
            vf_ref[l] = vf[:, 0:KM]
            for t in range(NV):
                vc_ref[l, t] = jnp.broadcast_to(vf[:, KM + t:KM + t + 1], (R, 128))
            vt = jnp.concatenate([vf[:, KM:D], jnp.zeros((R, 128 - (D - KM)), F32)], axis=1)
            vt = jnp.concatenate([vt, jnp.zeros((128 - R, 128), F32)], axis=0).T
            wt = _mm(vt[NV:D - KM, 0:R], ubuf[l], (((1,), (1,)), ((), ())))
            bb_ref[l] = jnp.broadcast_to(bbuf[...].astype(F32)[l:l + 1, :], (128, D)).T
            wt = jnp.concatenate([jnp.zeros((R, D), F32), wt], axis=0).T
            uf = jnp.concatenate([ubuf[l].astype(F32), jnp.zeros((D, 128 - R), F32)], axis=1)
            uw = jnp.where(lax.broadcasted_iota(jnp.int32, (D, 128), 1) < R, uf, wt)
            uw_ref[l] = pltpu.bitcast(uw.astype(BF16), U32)

        def load_x(c, s, l, n, r0, r1):
            if l == 0:
                return xin[c, r0:r1, n * 128:(n + 1) * 128]
            return xs_refs[s][(l - 1) % 2][ir, n, r0:r1, :]

        def down(c, s, l):
            zs = []
            for n in range(NT):
                xt = load_x(c, s, l, n, KM, D).astype(F32)
                bc = [jnp.broadcast_to(xt[t:t + 1, :], (8, 128)) for t in range(NV)]
                ps = [_mm(vf_ref[l, :, k * 128:(k + 1) * 128],
                          load_x(c, s, l, n, k * 128, (k + 1) * 128).astype(BF16)) for k in range(3)]
                hs = []
                for r in range(0, R, 8):
                    a = None
                    for t in range(NV):
                        q = vc_ref[l, t, r:r + 8, :] * bc[t]
                        a = q if a is None else a + q
                    hs.append(((ps[0][r:r + 8] + ps[1][r:r + 8]) + ps[2][r:r + 8]) + a)
                zs.append(jnp.concatenate(hs + [xt[NV:]], axis=0).astype(BF16))
            return zs

        def up(c, s, l, zs):
            w = pltpu.bitcast(uw_ref[l], BF16)
            gs = [_mm(w, zs[n]) for n in range(NT)]
            for r0 in range(0, D, 16):
                r1 = r0 + 16
                x0w = xin[c, r0:r1, :].astype(F32)
                outs = []
                for n in range(NT):
                    x0v = x0w[:, n * 128:(n + 1) * 128]
                    xv = x0v if l == 0 else load_x(c, s, l, n, r0, r1)
                    xn = x0v * (gs[n][r0:r1, :] + bb_ref[l, r0:r1, :]) + xv
                    if l == L - 1:
                        outs.append(xn)
                    else:
                        xs_refs[s][l % 2][iw, n, r0:r1, :] = xn
                if l == L - 1:
                    xout[c, r0:r1, :] = jnp.concatenate(outs, axis=1).astype(BF16)
                    if r1 in obounds:
                        out_copy(c, obounds.index(r1) - 1).start()

        def run(c0, pairs, hook):
            for p in range(pairs):
                for l in range(L):
                    if p == 0:
                        hook(l)
                    zs = [down(c0 + 2 * p + s, s, l) for s in range(2)]
                    for s in range(2):
                        up(c0 + 2 * p + s, s, l, zs[s])

        @pl.when(step == 0)
        def _():
            def hook(l):
                if l == 0:
                    for cp in group0:
                        cp.wait()
                    for cp in group1:
                        cp.start()
                if l == W2:
                    for cp in group1:
                        cp.wait()
                    for j in range(nb):
                        in_copy(nf + j, isem.at[1]).start()
                prep(l)
            run(0, FIRST, hook)

        @pl.when(step > 0)
        def _():
            c0 = nf + (step - 1) * nb
            for j in range(nb):
                in_copy(c0 + j, isem.at[step % 2]).wait()

            def hook(l):
                if l == 1:
                    for j in range(nb):
                        in_copy(c0 + nb + j, isem.at[(step + 1) % 2]).start()
            run(c0, BODY, hook)

        @pl.when(step == nsteps - 1)
        def _():
            pltpu.make_async_copy(xout, xout, osem.at[0]).wait()
            for j in range(nb):
                in_copy(NC + j, isem.at[nsteps % 2]).wait()

    any_spec = pl.BlockSpec(memory_space=pl.ANY)
    out = pl.pallas_call(
        kernel,
        grid=(nsteps,),
        in_specs=[any_spec] * 4,
        out_specs=any_spec,
        out_shape=jax.ShapeDtypeStruct((D, B), x0.dtype),
        scratch_shapes=[pltpu.VMEM((1, NT, D, 128), F32)] * 4 + [
            pltpu.VMEM((NC + nb, D, CN), BF16),
            pltpu.VMEM((NC, D, CN), BF16),
            pltpu.VMEM((L, D, R), BF16),
            pltpu.VMEM((L, R, D), BF16),
            pltpu.VMEM((L, R, KM), F32),
            pltpu.VMEM((L, D // 2, 128), U32),
            pltpu.VMEM((L, NV, R, 128), F32),
            pltpu.VMEM((L, D, 128), F32),
            pltpu.VMEM((L, D), BF16),
            pltpu.SMEM((2,), jnp.int32),
            pltpu.SemaphoreType.DMA((2,)),
            pltpu.SemaphoreType.DMA((1,)),
            pltpu.SemaphoreType.DMA((2,)),
        ],
        compiler_params=pltpu.CompilerParams(
            dimension_semantics=("arbitrary",), vmem_limit_bytes=64 * 1024 * 1024),
    )(x0.T, U, V, bs)
    return out.T
```

```python
import jax
import jax.numpy as jnp
from jax import lax
import jax.experimental.pallas as pl
import jax.experimental.pallas.tpu as pltpu

F32, BF16, U32 = jnp.float32, jnp.bfloat16, jnp.uint32

LANES = 128
TILES = 4
CHUNK = TILES * LANES
PAIRS = 3
OUT_ROWS = 32


def _mm(a, b, dims=(((1,), (0,)), ((), ()))):
    return lax.dot_general(a, b, dims, preferred_element_type=F32)


@jax.jit
def pallas_standalone__cross_network_dcn_v2__recsys_kernel(
    x0: jax.Array,
    U: jax.Array,
    V: jax.Array,
    bs: jax.Array,
):
    B, D = x0.shape
    L, _, R = U.shape
    KM = D // LANES * LANES
    NV = D - KM - (LANES - R)
    NC = B // CHUNK
    steps = 1 + (NC - 2) // (2 * PAIRS)
    assert B == (2 + (steps - 1) * 2 * PAIRS) * CHUNK and steps > 1
    assert 0 < NV and NV % 8 == 0 and R % 8 == 0 and (D - KM) % OUT_ROWS == 0 and L > 2

    SPLIT = KM // 2 // OUT_ROWS * OUT_ROWS
    FIRST, SECOND = ((KM, D), (0, SPLIT)), ((SPLIT, KM),)
    WHOLE = ((KM, D), (0, KM))

    def kernel(x_hbm, u_hbm, v_hbm, b_hbm, o_hbm,
               xa0, xa1, xb0, xb1, xin, xout, ubuf, vbuf, vf_ref, uw_ref, vc_ref, bias_ref, bbuf,
               zero_ref, in_sem, out_sem, start_sem):
        state = ((xa0, xa1), (xb0, xb1))
        step = pl.program_id(0)

        def columns(c):
            return pl.ds(pl.multiple_of(c * CHUNK, CHUNK), CHUNK)

        def in_copy(c, sem):
            src = min(c, NC - 1) if isinstance(c, int) else jnp.minimum(c, NC - 1)
            return pltpu.make_async_copy(x_hbm.at[:, columns(src)], xin.at[c], sem)

        def layer_copy(src, dst, l0, l1, sem):
            return pltpu.make_async_copy(src.at[l0:l1], dst.at[l0:l1], sem)

        start_copies = (
            (layer_copy(v_hbm, vbuf, 0, 1, start_sem.at[0]), in_copy(0, start_sem.at[0])),
            (layer_copy(u_hbm, ubuf, 0, 1, start_sem.at[1]),
             pltpu.make_async_copy(b_hbm, bbuf, start_sem.at[1])),
            (in_copy(1, start_sem.at[2]), layer_copy(v_hbm, vbuf, 1, 2, start_sem.at[2]),
             layer_copy(u_hbm, ubuf, 1, 2, start_sem.at[2])),
            (layer_copy(v_hbm, vbuf, 2, L, start_sem.at[3]),
             layer_copy(u_hbm, ubuf, 2, L, start_sem.at[3])),
        )

        @pl.when(step == 0)
        def _():
            for copies in start_copies:
                for copy in copies:
                    copy.start()
            zero_ref[0] = 0
            zero_ref[1] = 0

        write_idx = zero_ref[0]
        read_idx = zero_ref[1]

        def prepare_down(l):
            v = vbuf[l].astype(F32)
            vf_ref[l] = v[:, 0:KM]
            for t in range(NV):
                vc_ref[l, t] = jnp.broadcast_to(v[:, KM + t:KM + t + 1], (R, LANES))

        def prepare_up(l):
            vt = vbuf[l].astype(F32)[:, KM:D]
            vt = jnp.concatenate([vt, jnp.zeros((R, LANES - (D - KM)), F32)], axis=1)
            vt = jnp.concatenate([vt, jnp.zeros((LANES - R, LANES), F32)], axis=0).T
            bias_ref[l] = jnp.broadcast_to(bbuf[...].astype(F32)[l:l + 1, :], (LANES, D)).T
            wt = _mm(vt[NV:D - KM, 0:R], ubuf[l], (((1,), (1,)), ((), ())))
            w = jnp.concatenate([jnp.zeros((R, D), F32), wt], axis=0).T
            u = jnp.concatenate([ubuf[l].astype(F32), jnp.zeros((D, LANES - R), F32)], axis=1)
            uw = jnp.where(lax.broadcasted_iota(jnp.int32, (D, LANES), 1) < R, u, w)
            uw = jnp.concatenate([uw[KM:D], uw[0:KM]], axis=0)
            uw_ref[l] = pltpu.bitcast(uw.astype(BF16), U32)

        def load_x(c, l, n, r0, r1):
            chunk, slot = c
            if l == 0:
                return xin[chunk, r0:r1, n * LANES:(n + 1) * LANES]
            return state[slot][(l - 1) % 2][read_idx, n, r0:r1, :]

        tails = {}
        hidden = {}

        def down(c, l):
            slot = c[1]
            for n in range(TILES):
                xt = tails.pop((slot, n), None)
                if xt is None:
                    xt = load_x(c, l, n, KM, D).astype(F32)
                rows = [jnp.broadcast_to(xt[t:t + 1, :], (8, LANES)) for t in range(NV)]
                parts = [_mm(vf_ref[l, :, k:k + LANES], load_x(c, l, n, k, k + LANES).astype(BF16))
                         for k in range(0, KM, LANES)]
                h = []
                for r in range(0, R, 8):
                    vpu = vc_ref[l, 0, r:r + 8, :] * rows[0]
                    for t in range(1, NV):
                        vpu = vpu + vc_ref[l, t, r:r + 8, :] * rows[t]
                    mxu = parts[0][r:r + 8]
                    for part in parts[1:]:
                        mxu = mxu + part[r:r + 8]
                    h.append(mxu + vpu)
                hidden[slot, n] = jnp.concatenate(h + [xt[NV:]], axis=0).astype(BF16)

        def up(c, l, segments, hand_over=False):
            chunk, slot = c
            q0 = (segments[0][0] - KM) % D
            q1 = q0 + sum(r1 - r0 for r0, r1 in segments)
            uw = pltpu.bitcast(uw_ref[l, q0 // 2:q1 // 2, :], BF16)
            g = [_mm(uw, hidden[slot, n]) for n in range(TILES)]
            if l == L - 1:
                segments = [(r, r + OUT_ROWS) for r0, r1 in segments for r in range(r0, r1, OUT_ROWS)]
            q = 0
            for r0, r1 in segments:
                x0_rows = xin[chunk, r0:r1, :].astype(F32)
                bias = bias_ref[l, r0:r1, :]
                new = []
                for n in range(TILES):
                    x0_tile = x0_rows[:, n * LANES:(n + 1) * LANES]
                    x = load_x(c, l, n, r0, r1) if l else x0_tile
                    new.append(x0_tile * (g[n][q:q + r1 - r0, :] + bias) + x)
                    if l < L - 1:
                        state[slot][l % 2][write_idx, n, r0:r1, :] = new[n]
                        if hand_over and r0 == KM:
                            tails[slot, n] = new[n]
                if l == L - 1:
                    xout[chunk, r0:r1, :] = jnp.concatenate(new, axis=1).astype(BF16)
                    pltpu.make_async_copy(
                        xout.at[chunk, r0:r1, :], o_hbm.at[r0:r1, columns(chunk)], out_sem.at[0]).start()
                q += r1 - r0

        @pl.when(step == 0)
        def _():
            a, b = (0, 0), (1, 1)

            def arrived(group):
                for copy in start_copies[group]:
                    copy.wait()

            arrived(0)
            prepare_down(0)
            down(a, 0)
            arrived(1)
            prepare_up(0)
            up(a, 0, WHOLE)
            arrived(2)
            down(b, 0)
            prepare_down(1)
            down(a, 1)
            prepare_up(1)
            up(b, 0, WHOLE)
            up(a, 1, WHOLE)
            down(b, 1)
            arrived(3)
            for j in range(2 * PAIRS):
                in_copy(2 + j, in_sem.at[1]).start()
            prepare_down(2)
            up(b, 1, FIRST)
            for l in range(2, L):
                prepare_up(l)
                down(a, l)
                up(b, l - 1, SECOND)
                up(a, l, FIRST)
                down(b, l)
                if l < L - 1:
                    prepare_down(l + 1)
                up(a, l, SECOND)
                up(b, l, FIRST if l < L - 1 else WHOLE)

        @pl.when(step > 0)
        def _():
            c0 = 2 + (step - 1) * 2 * PAIRS
            for j in range(2 * PAIRS):
                in_copy(c0 + j, in_sem.at[step % 2]).wait()
            pending = None
            for p in range(PAIRS):
                a, b = (c0 + 2 * p, 0), (c0 + 2 * p + 1, 1)
                for l in range(L):
                    down(a, l)
                    if pending is None:
                        down(b, l)
                        up(a, l, WHOLE, hand_over=True)
                    else:
                        up(*pending, SECOND)
                        up(a, l, FIRST, hand_over=True)
                        down(b, l)
                        up(a, l, SECOND)
                    up(b, l, WHOLE if (p, l) == (PAIRS - 1, L - 1) else FIRST, hand_over=True)
                    pending = (b, l)
                    if l == 0:
                        for j in range(2):
                            in_copy(c0 + 2 * PAIRS + 2 * p + j, in_sem.at[(step + 1) % 2]).start()

        @pl.when(step == steps - 1)
        def _():
            pltpu.make_async_copy(xout, xout, out_sem.at[0]).wait()
            for j in range(2 * PAIRS):
                in_copy(NC + j, in_sem.at[steps % 2]).wait()

    any_spec = pl.BlockSpec(memory_space=pl.ANY)
    out = pl.pallas_call(
        kernel,
        grid=(steps,),
        in_specs=[any_spec] * 4,
        out_specs=any_spec,
        out_shape=jax.ShapeDtypeStruct((D, B), x0.dtype),
        scratch_shapes=[pltpu.VMEM((1, TILES, D, LANES), F32)] * 4 + [
            pltpu.VMEM((NC + 2 * PAIRS, D, CHUNK), BF16),
            pltpu.VMEM((NC, D, CHUNK), BF16),
            pltpu.VMEM((L, D, R), BF16),
            pltpu.VMEM((L, R, D), BF16),
            pltpu.VMEM((L, R, KM), F32),
            pltpu.VMEM((L, D // 2, LANES), U32),
            pltpu.VMEM((L, NV, R, LANES), F32),
            pltpu.VMEM((L, D, LANES), F32),
            pltpu.VMEM((L, D), BF16),
            pltpu.SMEM((2,), jnp.int32),
            pltpu.SemaphoreType.DMA((2,)),
            pltpu.SemaphoreType.DMA((1,)),
            pltpu.SemaphoreType.DMA((4,)),
        ],
        compiler_params=pltpu.CompilerParams(
            dimension_semantics=("arbitrary",),
            vmem_limit_bytes=64 * 1024 * 1024,
            disable_bounds_checks=True,
        ),
    )(x0.T, U, V, bs)
    return out.T
```

```python
import jax
import jax.numpy as jnp
from jax import lax
import jax.experimental.pallas as pl
import jax.experimental.pallas.tpu as pltpu

F32, BF16, U32 = jnp.float32, jnp.bfloat16, jnp.uint32

LANES = 128
TILES = 4
CHUNK = TILES * LANES
PAIRS = 3
OUT_ROWS = 32


def _mm(a, b, dims=(((1,), (0,)), ((), ()))):
    return lax.dot_general(a, b, dims, preferred_element_type=F32)


@jax.jit
def pallas_standalone__cross_network_dcn_v2__recsys_kernel(
    x0: jax.Array,
    U: jax.Array,
    V: jax.Array,
    bs: jax.Array,
):
    B, D = x0.shape
    L, _, R = U.shape
    KM = D // LANES * LANES
    NV = D - KM - (LANES - R)
    NC = B // CHUNK
    steps = 1 + (NC - 2) // (2 * PAIRS)
    assert B == (2 + (steps - 1) * 2 * PAIRS) * CHUNK and steps > 1
    assert 0 < NV and NV % 8 == 0 and R % 8 == 0 and (D - KM) % OUT_ROWS == 0 and L > 2

    SPLIT = KM // 2 // OUT_ROWS * OUT_ROWS
    FIRST, SECOND = ((KM, D), (0, SPLIT)), ((SPLIT, KM),)
    WHOLE = ((KM, D), (0, KM))

    def kernel(x_hbm, u_hbm, v_hbm, b_hbm, o_hbm,
               xa0, xa1, xb0, xb1, xin, xout, ubuf, vbuf, vf_ref, uw_ref, vc_ref, bias_ref, bbuf,
               zero_ref, in_sem, out_sem, start_sem):
        state = ((xa0, xa1), (xb0, xb1))
        step = pl.program_id(0)

        def columns(c):
            return pl.ds(pl.multiple_of(c * CHUNK, CHUNK), CHUNK)

        def in_copy(c, sem):
            src = min(c, NC - 1) if isinstance(c, int) else jnp.minimum(c, NC - 1)
            return pltpu.make_async_copy(x_hbm.at[:, columns(src)], xin.at[c], sem)

        def layer_copy(src, dst, l0, l1, sem):
            return pltpu.make_async_copy(src.at[l0:l1], dst.at[l0:l1], sem)

        start_copies = (
            (layer_copy(v_hbm, vbuf, 0, 1, start_sem.at[0]), in_copy(0, start_sem.at[0])),
            (layer_copy(u_hbm, ubuf, 0, 1, start_sem.at[1]),
             pltpu.make_async_copy(b_hbm, bbuf, start_sem.at[1])),
            (in_copy(1, start_sem.at[2]), layer_copy(v_hbm, vbuf, 1, 2, start_sem.at[2]),
             layer_copy(u_hbm, ubuf, 1, 2, start_sem.at[2])),
            (layer_copy(v_hbm, vbuf, 2, L, start_sem.at[3]),
             layer_copy(u_hbm, ubuf, 2, L, start_sem.at[3])),
        )

        @pl.when(step == 0)
        def _():
            for copies in start_copies:
                for copy in copies:
                    copy.start()
            zero_ref[0] = 0
            zero_ref[1] = 0

        write_idx = zero_ref[0]
        read_idx = zero_ref[1]

        def prepare_down(l):
            v = vbuf[l].astype(F32)
            vf_ref[l] = v[:, 0:KM]
            for t in range(NV):
                vc_ref[l, t] = jnp.broadcast_to(v[:, KM + t:KM + t + 1], (R, LANES))

        def prepare_up(l):
            vt = vbuf[l].astype(F32)[:, KM:D]
            vt = jnp.concatenate([vt, jnp.zeros((R, LANES - (D - KM)), F32)], axis=1)
            vt = jnp.concatenate([vt, jnp.zeros((LANES - R, LANES), F32)], axis=0).T
            bias_ref[l] = jnp.broadcast_to(bbuf[...].astype(F32)[l:l + 1, :], (LANES, D)).T
            wt = _mm(vt[NV:D - KM, 0:R], ubuf[l], (((1,), (1,)), ((), ())))
            w = jnp.concatenate([jnp.zeros((R, D), F32), wt], axis=0).T
            u = jnp.concatenate([ubuf[l].astype(F32), jnp.zeros((D, LANES - R), F32)], axis=1)
            uw = jnp.where(lax.broadcasted_iota(jnp.int32, (D, LANES), 1) < R, u, w)
            uw = jnp.concatenate([uw[KM:D], uw[0:KM]], axis=0)
            uw_ref[l] = pltpu.bitcast(uw.astype(BF16), U32)

        def load_x(c, l, n, r0, r1):
            chunk, slot = c
            if l == 0:
                return xin[chunk, r0:r1, n * LANES:(n + 1) * LANES]
            return state[slot][(l - 1) % 2][read_idx, n, r0:r1, :]

        tails = {}
        hidden = {}

        def down(c, l):
            slot = c[1]
            for n in range(TILES):
                xt = tails.pop((slot, n), None)
                if xt is None:
                    xt = load_x(c, l, n, KM, D).astype(F32)
                vpu = vc_ref[l, 0] * xt[0:1, :]
                for t in range(1, NV):
                    vpu = vpu + vc_ref[l, t] * xt[t:t + 1, :]
                mxu = None
                for k in range(0, KM, LANES):
                    part = _mm(vf_ref[l, :, k:k + LANES], load_x(c, l, n, k, k + LANES).astype(BF16))
                    mxu = part if mxu is None else mxu + part
                hidden[slot, n] = jnp.concatenate([mxu + vpu, xt[NV:]], axis=0).astype(BF16)

        def up(c, l, segments, hand_over=False):
            chunk, slot = c
            q0 = (segments[0][0] - KM) % D
            q1 = q0 + sum(r1 - r0 for r0, r1 in segments)
            uw = pltpu.bitcast(uw_ref[l, q0 // 2:q1 // 2, :], BF16)
            g = [_mm(uw, hidden[slot, n]) for n in range(TILES)]
            if l == L - 1:
                segments = [(r, r + OUT_ROWS) for r0, r1 in segments for r in range(r0, r1, OUT_ROWS)]
            q = 0
            for r0, r1 in segments:
                x0_rows = xin[chunk, r0:r1, :].astype(F32)
                bias = bias_ref[l, r0:r1, :]
                new = []
                for n in range(TILES):
                    x0_tile = x0_rows[:, n * LANES:(n + 1) * LANES]
                    x = load_x(c, l, n, r0, r1) if l else x0_tile
                    new.append(x0_tile * (g[n][q:q + r1 - r0, :] + bias) + x)
                    if l < L - 1:
                        state[slot][l % 2][write_idx, n, r0:r1, :] = new[n]
                        if hand_over and r0 == KM:
                            tails[slot, n] = new[n]
                if l == L - 1:
                    xout[chunk, r0:r1, :] = jnp.concatenate(new, axis=1).astype(BF16)
                    pltpu.make_async_copy(
                        xout.at[chunk, r0:r1, :], o_hbm.at[r0:r1, columns(chunk)], out_sem.at[0]).start()
                q += r1 - r0

        @pl.when(step == 0)
        def _():
            a, b = (0, 0), (1, 1)

            def arrived(group):
                for copy in start_copies[group]:
                    copy.wait()

            arrived(0)
            prepare_down(0)
            down(a, 0)
            arrived(1)
            prepare_up(0)
            up(a, 0, WHOLE)
            arrived(2)
            down(b, 0)
            prepare_down(1)
            down(a, 1)
            prepare_up(1)
            up(b, 0, WHOLE)
            up(a, 1, WHOLE)
            down(b, 1)
            arrived(3)
            for j in range(2 * PAIRS):
                in_copy(2 + j, in_sem.at[1]).start()
            prepare_down(2)
            up(b, 1, FIRST)
            for l in range(2, L):
                prepare_up(l)
                down(a, l)
                up(b, l - 1, SECOND)
                up(a, l, FIRST)
                down(b, l)
                if l < L - 1:
                    prepare_down(l + 1)
                up(a, l, SECOND)
                up(b, l, FIRST if l < L - 1 else WHOLE)

        @pl.when(step > 0)
        def _():
            c0 = 2 + jnp.maximum(step - 1, 0) * 2 * PAIRS
            for j in range(2 * PAIRS):
                in_copy(c0 + j, in_sem.at[step % 2]).wait()
            pending = None
            for p in range(PAIRS):
                a, b = (c0 + 2 * p, 0), (c0 + 2 * p + 1, 1)
                for l in range(L):
                    down(a, l)
                    if pending is None:
                        down(b, l)
                        up(a, l, WHOLE, hand_over=True)
                    else:
                        up(*pending, SECOND)
                        up(a, l, FIRST, hand_over=True)
                        down(b, l)
                        up(a, l, SECOND)
                    up(b, l, WHOLE if (p, l) == (PAIRS - 1, L - 1) else FIRST, hand_over=True)
                    pending = (b, l)
                    if l == 0:
                        for j in range(2):
                            in_copy(c0 + 2 * PAIRS + 2 * p + j, in_sem.at[(step + 1) % 2]).start()

        @pl.when(step == steps - 1)
        def _():
            pltpu.make_async_copy(xout, xout, out_sem.at[0]).wait()
            for j in range(2 * PAIRS):
                in_copy(NC + j, in_sem.at[steps % 2]).wait()

    any_spec = pl.BlockSpec(memory_space=pl.ANY)
    out = pl.pallas_call(
        kernel,
        grid=(steps,),
        in_specs=[any_spec] * 4,
        out_specs=any_spec,
        out_shape=jax.ShapeDtypeStruct((D, B), x0.dtype),
        scratch_shapes=[pltpu.VMEM((1, TILES, D + 8, LANES), F32)] * 4 + [
            pltpu.VMEM((NC + 2 * PAIRS, D, CHUNK), BF16),
            pltpu.VMEM((NC, D, CHUNK), BF16),
            pltpu.VMEM((L, D, R), BF16),
            pltpu.VMEM((L, R, D), BF16),
            pltpu.VMEM((L, R, KM), F32),
            pltpu.VMEM((L, D // 2, LANES), U32),
            pltpu.VMEM((L, NV, R, LANES), F32),
            pltpu.VMEM((L, D, LANES), F32),
            pltpu.VMEM((L, D), BF16),
            pltpu.SMEM((2,), jnp.int32),
            pltpu.SemaphoreType.DMA((2,)),
            pltpu.SemaphoreType.DMA((1,)),
            pltpu.SemaphoreType.DMA((4,)),
        ],
        compiler_params=pltpu.CompilerParams(
            dimension_semantics=("arbitrary",),
            vmem_limit_bytes=64 * 1024 * 1024,
        ),
    )(x0.T, U, V, bs)
    return out.T
```
